```python
import os as _os
_os.environ.setdefault("JAX_PLATFORMS", "cpu")
import jax
import jax.numpy as jnp

def _softmax(x, axis=-1):
    return jax.nn.softmax(x, axis=axis)
def _gelu(x):
    return jax.nn.gelu(x, approximate=True)
def _silu(x):
    return jax.nn.silu(x)
def _sigmoid(x):
    return jax.nn.sigmoid(x)
def _layernorm(x, axis=-1, eps=1e-5):
    m = jnp.mean(x, axis=axis, keepdims=True)
    v = jnp.var(x, axis=axis, keepdims=True)
    return (x - m) / jnp.sqrt(v + eps)
def _scatter_add(tgt, idx, src, axis=0):
    return tgt.at[idx].add(src)
def _segment_sum(src, seg, n):
    return jax.ops.segment_sum(src, seg, n)
class _Rng:
    def __init__(self, key):
        self._k = key
    def _next(self):
        self._k, sub = jax.random.split(self._k)
        return sub
    def normal(self, shape):
        return jax.random.normal(self._next(), shape, dtype=jnp.bfloat16)
    def randint(self, lo, hi, shape):
        return jax.random.randint(self._next(), shape, lo, hi, dtype=jnp.int32)
    def uniform(self, shape, lo=0.0, hi=1.0):
        return jax.random.uniform(self._next(), shape, jnp.bfloat16, lo, hi)
    def permutation(self, n):
        return jax.random.permutation(self._next(), n)


kernel_name = 'parallel_sum__sliding_local_dilated__glu_gated_reglu__prompt'

def setup_inputs():
    _rng = _Rng(jax.random.key(int.from_bytes(__import__("os").urandom(4), "little")))
    _w = (lambda a: (lambda t: t.astype(jnp.bfloat16) if jnp.issubdtype(t.dtype, jnp.floating) else t)(jnp.asarray(a)))
    def _A_setup():
        B, S, D = 1, 2048, 576
        return {
            "x": _w((lambda *s: _rng.normal(s) * 0.05)(B, S, D)),
            "wqkv": _w((lambda *s: _rng.normal(s) * 0.05)(D, 3 * D)),
            "wo": _w((lambda *s: _rng.normal(s) * 0.05)(D, D)),
        }
    _A_in = _A_setup()

    def _B_setup():
        B, S, D, F = 1, 2048, 576, 4608
        return {
            "x": _w((lambda *s: _rng.normal(s) * 0.05)(B, S, D)),
            "W_gate": _w((lambda *s: _rng.normal(s) * 0.1)(D, F) * (2.0 / D) ** 0.5),
            "W_up": _w((lambda *s: _rng.normal(s) * 0.1)(D, F) * (2.0 / D) ** 0.5),
            "W_down": _w((lambda *s: _rng.normal(s) * 0.1)(F, D) * (1.0 / F) ** 0.5),
        }
    _B_in = _B_setup()

    return {
        "A_x": _A_in["x"],
        "A_wqkv": _A_in["wqkv"],
        "A_wo": _A_in["wo"],
        "B_x": _B_in["x"],
        "B_W_gate": _B_in["W_gate"],
        "B_W_up": _B_in["W_up"],
        "B_W_down": _B_in["W_down"],
    }

def reference(A_x, A_wqkv, A_wo, B_x, B_W_gate, B_W_up, B_W_down):
    def _A_ref(x, wqkv, wo):
        B, S, D = x.shape
        H = 32; Dh = D // H
        W, dil = 8, 2
        qkv = (lambda x, *d: x.transpose(*d))((x @ wqkv).reshape(B, S, 3, H, Dh), 2, 0, 3, 1, 4)
        q, k, v = qkv[0], qkv[1], qkv[2]
        scale = Dh ** -0.5
        pos = jnp.arange(S)
        off = jnp.arange(W) * dil
        idx = pos[:, None] - off[None, :]
        mask = idx >= 0
        idx_c = jnp.where(mask, idx, 0).reshape(-1)
        kg = k[:, :, idx_c, :].reshape(B, H, S, W, Dh)
        vg = v[:, :, idx_c, :].reshape(B, H, S, W, Dh)
        logits = jnp.einsum("bhsd,bhswd->bhsw", q, kg) * scale
        logits = jnp.where(mask[None, None, :, :], logits, -1e9)
        attn = _softmax(logits, axis=-1)
        o = jnp.einsum("bhsw,bhswd->bhsd", attn, vg)
        return (lambda x, *d: x.transpose(*d))(o, 0, 2, 1, 3).reshape(B, S, D) @ wo

    def _B_ref(x, W_gate, W_up, W_down):
        gate = jnp.einsum("bsd,df->bsf", x, W_gate)
        up = jnp.einsum("bsd,df->bsf", x, W_up)
        gate = gate * (lambda x, dt: x.astype(dt))(gate > 0, gate.dtype)
        h = gate * up
        return jnp.einsum("bsf,fd->bsd", h, W_down)

    x = A_x
    xn = _layernorm(x, axis=-1)
    return x + _A_ref(xn, A_wqkv, A_wo) + _B_ref(xn, B_W_gate, B_W_up, B_W_down)
```

```python
import jax
import jax.numpy as jnp
from jax import lax
import jax.experimental.pallas as pl
import jax.experimental.pallas.tpu as pltpu

S, D, F = 2048, 576, 4608
H, DH = 32, 18
W, DIL = 8, 2
EPS = 1e-5
FC = 512
TC = 512
NT = S // 128

f32 = jnp.float32
bf16 = jnp.bfloat16
_NN = (((1,), (0,)), ((), ()))
_NT = (((1,), (1,)), ((), ()))


def _dot(a, b, dn=_NN):
    return lax.dot_general(a, b, dn, preferred_element_type=f32)


def _kernel(x_hbm, wqkv_hbm, wo_hbm, wg_hbm, wu_hbm, wd_hbm, out_hbm,
            x_v, wqkv_v, wo_v, wg_v, wu_v, wd_v, out_v,
            xn_v, wqkvT_v, woT_v, qkv_v, o_v, acc_v,
            x_sem, w_sem, f_sem, o_sem):
    NF = F // FC
    NC = S // TC

    def x_copy(c):
        return pltpu.make_async_copy(x_hbm.at[:, pl.ds(c * TC, TC)], x_v.at[c], x_sem.at[c])

    def f_copies(i):
        off = pl.multiple_of(i * FC, FC) if not isinstance(i, int) else i * FC
        return [
            pltpu.make_async_copy(wg_hbm.at[:, pl.ds(off, FC)], wg_v.at[i], f_sem.at[3 * i]),
            pltpu.make_async_copy(wu_hbm.at[:, pl.ds(off, FC)], wu_v.at[i], f_sem.at[3 * i + 1]),
            pltpu.make_async_copy(wd_hbm.at[:, pl.ds(off, FC)], wd_v.at[i], f_sem.at[3 * i + 2]),
        ]

    wqkv_copy = pltpu.make_async_copy(wqkv_hbm, wqkv_v, w_sem.at[0])
    wo_copy = pltpu.make_async_copy(wo_hbm, wo_v, w_sem.at[1])

    def o_copy(c):
        return pltpu.make_async_copy(out_v.at[c], out_hbm.at[:, pl.ds(c * TC, TC)], o_sem.at[c])

    wqkv_copy.start()
    x_copy(0).start()
    wqkv_copy.wait()
    for c in range(1, NC):
        x_copy(c).start()
    wo_copy.start()
    for cp in f_copies(0):
        cp.start()

    wqkvT_v[...] = wqkv_v[...].astype(f32).T.astype(bf16)

    for c in range(NC):
        x_copy(c).wait()
        x = x_v[c].astype(f32)
        mean = jnp.sum(x, axis=0, keepdims=True) * (1.0 / D)
        xc = x - mean
        var = jnp.sum(xc * xc, axis=0, keepdims=True) * (1.0 / D)
        xn = xc * lax.rsqrt(var + EPS)
        xn_v[pl.ds(c * TC, TC), :] = xn.T.astype(bf16)
        qkv = _dot(wqkvT_v[...], xn.astype(bf16))
        for j in range(TC // 128):
            qkv_v[1 + c * (TC // 128) + j] = qkv[:, j * 128:(j + 1) * 128]
        acc_v[:, pl.ds(c * TC, TC)] = x
        if c == 0:
            qkv_v[0] = jnp.broadcast_to(qkv[:, 0:1], (3 * D, 128))

    wo_copy.wait()
    woT_v[...] = wo_v[...].astype(f32).T.astype(bf16)

    def attention(t, g):
        lane = lax.broadcasted_iota(jnp.int32, (8, 128), 1)
        keep = [lane < 128 - DIL * w for w in range(W)]

        def rows(part, d):
            return pl.ds(part * D + g * 8 * DH + d, 8, stride=DH)

        def windows(part, d):
            cur = qkv_v[t + 1, rows(part, d), :]
            prev = qkv_v[t, rows(part, d), :]
            return [cur] + [pltpu.roll(jnp.where(keep[w], cur, prev), DIL * w, 1) for w in range(1, W)]

        lg = [None] * W
        for d in range(DH):
            q = qkv_v[t + 1, rows(0, d), :]
            ks = windows(1, d)
            for w in range(W):
                lg[w] = q * ks[w] if d == 0 else lg[w] + q * ks[w]
        pos = lane + t * 128
        lg = [jnp.where(pos >= DIL * w, lg[w] * (DH ** -0.5), -1e9) for w in range(W)]
        m = lg[0]
        for w in range(1, W):
            m = jnp.maximum(m, lg[w])
        e = [jnp.exp(l - m) for l in lg]
        s = e[0]
        for w in range(1, W):
            s = s + e[w]
        r = 1.0 / s
        p = [ew * r for ew in e]
        for d in range(DH):
            vs = windows(2, d)
            o = p[0] * vs[0]
            for w in range(1, W):
                o = o + p[w] * vs[w]
            o_v[t, rows(0, d), :] = o

    TPI = -(-NT // NF)

    def ffn_step(i, carry):
        @pl.when(i + 1 < NF)
        def _():
            for cp in f_copies(i + 1):
                cp.start()
        for cp in f_copies(i):
            cp.wait()
        att = [(jnp.minimum(i * TPI + j, NT - TPI + j), g) for j in range(TPI) for g in range(4)]
        MB = 512
        nb = S // MB
        for b in range(nb):
            xn = xn_v[pl.ds(b * MB, MB), :]
            gate = _dot(xn, wg_v[i])
            up = _dot(xn, wu_v[i])
            h = (jnp.maximum(gate, 0.0) * up).astype(bf16)
            for t, g in att[b * len(att) // nb:(b + 1) * len(att) // nb]:
                attention(t, g)
            acc_v[:, pl.ds(b * MB, MB)] += _dot(wd_v[i], h, _NT)
        return carry

    lax.fori_loop(0, NF, ffn_step, 0)

    for c in range(NC):
        o = jnp.concatenate([o_v[c * (TC // 128) + j] for j in range(TC // 128)], axis=1).astype(bf16)
        out_v[c] = (acc_v[:, pl.ds(c * TC, TC)] + _dot(woT_v[...], o)).astype(bf16)
        o_copy(c).start()
    for c in range(NC):
        o_copy(c).wait()


@jax.jit
def pallas_parallel_sum__sliding_local_dilated__glu_gated_reglu__prompt_kernel(
    A_x, A_wqkv, A_wo, B_x, B_W_gate, B_W_up, B_W_down,
):
    NF, NC = F // FC, S // TC
    out_t = pl.pallas_call(
        _kernel,
        out_shape=jax.ShapeDtypeStruct((D, S), bf16),
        in_specs=[pl.BlockSpec(memory_space=pl.ANY)] * 6,
        out_specs=pl.BlockSpec(memory_space=pl.ANY),
        scratch_shapes=[
            pltpu.VMEM((NC, D, TC), bf16),
            pltpu.VMEM((D, 3 * D), bf16),
            pltpu.VMEM((D, D), bf16),
            pltpu.VMEM((NF, D, FC), bf16),
            pltpu.VMEM((NF, D, FC), bf16),
            pltpu.VMEM((NF, D, FC), bf16),
            pltpu.VMEM((NC, D, TC), bf16),
            pltpu.VMEM((S, D), bf16),
            pltpu.VMEM((3 * D, D), bf16),
            pltpu.VMEM((D, D), bf16),
            pltpu.VMEM((NT + 1, 3 * D, 128), f32),
            pltpu.VMEM((NT, D, 128), f32),
            pltpu.VMEM((D, S), f32),
            pltpu.SemaphoreType.DMA((NC,)),
            pltpu.SemaphoreType.DMA((2,)),
            pltpu.SemaphoreType.DMA((3 * NF,)),
            pltpu.SemaphoreType.DMA((NC,)),
        ],
        compiler_params=pltpu.CompilerParams(vmem_limit_bytes=110 * 2**20),
        name="fused_block",
    )(A_x[0].T, A_wqkv, A_wo, B_W_gate, B_W_up, B_W_down.T)
    return out_t.T[None]
```

```python
from functools import partial

import numpy as np
import jax
import jax.numpy as jnp
from jax import lax
import jax.experimental.pallas as pl
import jax.experimental.pallas.tpu as pltpu

S, D, F = 2048, 576, 4608
H, DH = 32, 18
W, DIL = 8, 2
EPS = 1e-5

T = 128
KB = 64
NK = D // KB
NQ = F // (4 * T)
NB = S // (4 * T)
NU = S // (2 * T)
DR = D // 4
GR = 64
PR = 96
RING = 4

f32, bf16, u32 = jnp.float32, jnp.bfloat16, jnp.uint32
_NN = (((1,), (0,)), ((), ()))
_NT = (((1,), (1,)), ((), ()))


def _unit(i, j):
    m = np.zeros((2, 2))
    m[i, j] = 1.0
    return m


_STRASSEN = [
    (_unit(0, 0) + _unit(1, 1), _unit(0, 0) + _unit(1, 1), _unit(0, 0) + _unit(1, 1)),
    (_unit(1, 0) + _unit(1, 1), _unit(0, 0), _unit(1, 0) - _unit(1, 1)),
    (_unit(0, 0), _unit(0, 1) - _unit(1, 1), _unit(0, 1) + _unit(1, 1)),
    (_unit(1, 1), _unit(1, 0) - _unit(0, 0), _unit(0, 0) + _unit(1, 0)),
    (_unit(0, 0) + _unit(0, 1), _unit(1, 1), _unit(0, 1) - _unit(0, 0)),
    (_unit(1, 0) - _unit(0, 0), _unit(0, 0) + _unit(0, 1), _unit(1, 1)),
    (_unit(0, 1) - _unit(1, 1), _unit(1, 0) + _unit(1, 1), _unit(0, 0)),
]

_PATTERNS = [np.array(p, float) for p in (
    [[1, 0], [1, 0]], [[1, 0], [2, 0]], [[2, 0], [1, 0]], [[1, 0], [0, 1]],
    [[0, 1], [0, 1]], [[0, 1], [0, 2]], [[0, 2], [0, 1]], [[2, 0], [0, 1]],
    [[1, -1], [0, 0]], [[2, -1], [0, 0]], [[0, 0], [1, -1]], [[0, 0], [2, -1]],
    [[1, 0], [0, 0]], [[1, 0], [0, 0]], [[0, 0], [0, 1]], [[0, 0], [0, 1]],
)]
DIAG = 12


def _build_passes():
    prods = []
    for n, scales in enumerate([(1, 1, 1), (2, .5, 2), (1, .5, 1), (.5, 1, 1)]):
        left, right, mid = (np.diag([1., s]) for s in scales)
        ileft, iright, imid = (np.diag([1., 1. / s]) for s in scales)
        for u, v, w in _STRASSEN:
            prods.append((2 * n, ileft @ u @ mid, imid @ v @ iright, left @ w @ right))
    for q in range(2):
        for column, dual in (((1, 2), (-1 / 3, 2 / 3)), ((2, 1), (2 / 3, -1 / 3))):
            u, w = np.zeros((2, 2)), np.zeros((2, 2))
            u[:, 0], w[:, q] = dual, column
            prods.append((8, u, _unit(0, q), w))
    passes = [[] for _ in _PATTERNS]
    for k0, u, v, w in prods:
        for pair, pat in zip(passes, _PATTERNS):
            scale = (w * pat).sum() / (pat * pat).sum()
            if len(pair) < 2 and np.array_equal(w, scale * pat):
                lead = v.ravel()[np.abs(v).argmax()]
                pair.append((
                    [(float(u[p, k] * scale * lead), p, k0 + k) for p in range(2) for k in range(2) if u[p, k]],
                    [(float(v[k, q] / lead), q, k0 + k) for k in range(2) for q in range(2) if v[k, q]]))
                break
    total = np.zeros((2, NK, NK, 2, 2, 2))
    for pair, pat in zip(passes, _PATTERNS):
        for a_terms, b_terms in pair:
            for ca, p, ka in a_terms:
                for cb, q, kb in b_terms:
                    total[p, ka, kb, q] += ca * cb * pat
    assert np.abs(total - np.einsum('pr,kl,qs->pklqrs', np.eye(2), np.eye(NK), np.eye(2))).max() < 1e-12
    return passes


_PASSES = _build_passes()


def _lincomb(terms):
    terms = sorted(terms, key=lambda t: (t[0] != 1, t[0] < 0))
    c, acc = terms[0]
    if c == 1 and len(terms) == 1:
        return acc
    acc = acc.astype(f32)
    if c != 1:
        acc = acc * float(c)
    for c, val in terms[1:]:
        val = val.astype(f32)
        if abs(c) != 1:
            val = val * float(abs(c))
        acc = acc + val if c > 0 else acc - val
    return acc


def _recombine(m, diag=None):
    p1, p2, p3, g = m(0), m(1), m(2), m(3)
    t = p1 + p2 + p3
    c00, c10 = t + p3, t + p2
    p1, p2, p3, g2 = m(4), m(5), m(6), m(7)
    t = p1 + p2 + p3
    g = g + g2
    c01, c11, c00 = t + p3, (t + p2) + g, c00 + (g + g2)
    if diag:
        e0, e1 = diag
        t0, q0, t1, q1 = m(8), m(9), m(10), m(11)
    else:
        e0, t0, q0 = m(12) + m(13), m(8), m(9)
        e1, t1, q1 = m(14) + m(15), m(10), m(11)
    t0, t1 = t0 + q0, t1 + q1
    return ((c00 + (t0 + q0)) + e0, c01 - t0), (c10 + (t1 + q1), (c11 - t1) + e1)


def _strassen_operand(side, i, block):
    cf = _STRASSEN[i][side]
    return _lincomb([(cf[a, b], block(a, b)) for a in range(2) for b in range(2) if cf[a, b]])


def _strassen2_operands(side, outer, block):
    sub = {(r, c): _strassen_operand(side, outer, lambda a, b: block(2 * a + r, 2 * b + c))
           for r in range(2) for c in range(2)}
    return [_strassen_operand(side, i, lambda a, b: sub[a, b]) for i in range(7)]


def _strassen_recombine(m):
    out = {}
    for i, (_, _, w) in enumerate(_STRASSEN):
        val = m(i)
        for key in ((0, 0), (0, 1), (1, 0), (1, 1)):
            if w[key] and key not in out:
                out[key] = val
            elif w[key]:
                out[key] = out[key] + val if w[key] > 0 else out[key] - val
    return out


class _Weaver:
    def __init__(self):
        self.jobs = []
        self.count = 0
        self.busy = False

    def add(self, pieces, ticks):
        self.jobs.append(dict(pieces=pieces, done=0, time=0, ticks=ticks))

    def tick(self, result=None, duration=1):
        for job in self.jobs:
            job['time'] += duration
            job['owed'] = job['time'] * len(job['pieces']) / job['ticks'] - job['done']
        lead = None if self.busy else max(self.jobs, key=lambda job: job['owed'], default=None)
        due = []
        for job in self.jobs:
            count = max(0, int(-(-job['owed'] // 1) if job is lead else job['owed'] // 1))
            due += job['pieces'][job['done']:job['done'] + count]
            job['done'] += count
        if result is not None:
            row = self.count % 4 * (result.shape[0] // 8) // 4 * 8
            for pace in dict.fromkeys(pace for _, pacers in due for pace in pacers):
                pace(result[row:row + 8])
        _run(due)
        self.jobs = [job for job in self.jobs if job['done'] < len(job['pieces'])]
        self.busy = bool(due)
        self.count += 1

    def drain(self):
        while self.jobs:
            self.tick()


def _run(pieces):
    for work, _ in pieces:
        work()


def _idle():
    pass


def _kernel(x_hbm, wqkv_hbm, wo_hbm, wg_hbm, wu_hbm, wd_hbm, out_hbm,
            x_v, w_v, qrem_v, orem_v, out_v,
            xc0_v, xc1_v, xe_v, wc_v, we_v, wd_v, hc_v, pc_v, oc_v, sx_v, sp_v,
            xn_v, h_v, qkv_v, o_v, y_v,
            zero_s, x_sem, w_sem, o_sem):
    weaver = _Weaver()
    xc_v = (xc0_v, xc1_v)
    zero_s[0] = 0

    def pacer(ref):
        def pace(value=None):
            spare = (0,) * (len(ref.shape) - 3) + (zero_s[0] + (ref.shape[-3] - 1),)
            value = jnp.zeros((8, T), f32) if value is None else value
            ref[(*spare, pl.ds(0, 8), pl.ds(0, T))] = (
                pltpu.bitcast(value, u32) if ref.dtype == u32 else value.astype(ref.dtype))
        return pace

    p_xc, p_xe = [pacer(r) for r in xc_v], pacer(xe_v)
    p_x, p_w, p_pc, p_oc, p_sx, p_sp, p_xn, p_h, p_qkv, p_o, p_y = (
        pacer(r) for r in (x_v, w_v, pc_v, oc_v, sx_v, sp_v, xn_v, h_v, qkv_v, o_v, y_v))

    def dot(a, b, dims=_NN):
        a, b = (pltpu.bitcast(val, bf16) if val.dtype == u32 else val for val in (a, b))
        out = lax.dot_general(a, b, dims, preferred_element_type=f32)
        weaver.tick(out, 0.5 if out.shape[0] == GR else 1)
        return out

    def tile(t, width=T):
        return pl.ds(t * width if isinstance(t, int) else pl.multiple_of(t * width, width), width)

    def least(a, b):
        return min(a, b) if isinstance(a, int) else jnp.minimum(a, b)

    def block_rows(k, part=0, size=KB):
        return pl.ds(k * KB + part * size, size)

    def put(ref, index, row, val):
        val = val.astype(bf16)
        if ref.dtype == u32:
            val, row = pltpu.bitcast(val, u32), row // 2
        ref[index, pl.ds(row, val.shape[0]), :] = val

    def x_copies(*pairs):
        return [pltpu.make_async_copy(x_hbm.at[:, tile(t)], x_v.at[t // 4, t % 4], x_sem.at[t // 2])
                for u in pairs for t in (2 * u, 2 * u + 1)]

    def w_copy(hbm, t, dst, sem):
        return pltpu.make_async_copy(hbm.at[:, tile(t)], w_v.at[dst], w_sem.at[sem])

    def gate_up_copies(i, fts, sem):
        return [w_copy(hbm, 4 * least(i, NQ - 1) + ft, (i & RING - 1, 4 * q + ft), sem)
                for ft in fts for q, hbm in enumerate((wg_hbm, wu_hbm))]

    def down_tile(i, n):
        return (RING + n // 2, 10 + n % 2) if isinstance(i, int) and i == 0 else (i & RING - 1, 8 + n)

    def down_copies(i, sem):
        return [w_copy(wd_hbm, 4 * least(i, NQ - 1) + n, down_tile(i, n), sem) for n in range(4)]

    def step_copies(i):
        c = i if isinstance(i, int) else jnp.where(i < 6, i, 9)
        sem = i & RING - 1
        return (gate_up_copies(i + 1, range(4), sem) + down_copies(i, sem)
                + [w_copy(wqkv_hbm, least(i, 5) + 6 * q, (RING + q, c), sem) for q in range(2)])

    def extra_copies(sem):
        return ([pltpu.make_async_copy(wqkv_hbm.at[:, pl.ds(12 * T, 3 * D - 12 * T)], qrem_v, w_sem.at[sem]),
                 pltpu.make_async_copy(wo_hbm.at[:, pl.ds(4 * T, D - 4 * T)], orem_v, w_sem.at[sem])]
                + down_copies(0, sem) + [w_copy(wqkv_hbm, 6 * q, (RING + q, 0), sem) for q in range(2)])

    def wo_copies(sem):
        return [w_copy(wo_hbm, 2 * q + c, (RING + q, 7 + c), sem) for q in range(2) for c in range(2)]

    def out_parts(n, q):
        return [(4 * T + 32 * q, 0, 32), (2 * T * q, 32, PR)] if n == 0 else [(2 * T * q + n - 32, 0, PR)]

    def out_copies(b, r, n):
        return [pltpu.make_async_copy(out_v.at[b, r, pl.ds(row, hi - lo)],
                                      out_hbm.at[pl.ds(row, hi - lo), tile(2 * b + r, 2 * T)], o_sem.at[0])
                for q in range(2) for row, lo, hi in out_parts(n, q)]

    def starts(copies):
        return [(cp.start, [p_w]) for cp in copies]

    def wait(copies):
        for cp in copies:
            cp.wait()

    def x_stats(u):
        st = {}

        def fold(val):
            return val.reshape(KB // 8, 8, T).sum(axis=0)

        def mean(k):
            for t in (2 * u, 2 * u + 1):
                part = fold(x_v[t // 4, t % 4, block_rows(k), :].astype(f32))
                st[t] = part if k == 0 else st[t] + part
                if k == NK - 1:
                    st['mean', t] = jnp.sum(st[t], axis=0, keepdims=True) * (1.0 / D)

        def variance(t, k):
            centred = x_v[t // 4, t % 4, block_rows(k), :].astype(f32) - st['mean', t]
            xn_v[t, block_rows(k), :] = centred
            part = fold(centred * centred)
            st[t] = part if k == 0 else st[t] + part
            if k == NK - 1:
                inv = lax.rsqrt(jnp.sum(st[t], axis=0, keepdims=True) * (1.0 / D) + EPS)
                xn_v[t, pl.ds(D, 16), :] = jnp.broadcast_to(inv, (16, T))

        return ([(partial(mean, k), [p_x]) for k in range(NK)]
                + [(partial(variance, t, k), [p_x]) for k in range(NK) for t in (2 * u, 2 * u + 1)])

    def normalised(t, k, s):
        return xn_v[t, block_rows(k, s, 16), :] * xn_v[t, pl.ds(D, 16), :]

    def pass_operands(side, load, dst, pacers, passes=range(16)):
        def piece(v, s):
            src = {(half, k): load(half, k, s) for half in range(2) for k in range(2 * v, min(2 * v + 2, NK))}
            for j in passes:
                for n, prod in enumerate(_PASSES[j]):
                    if prod[side][0][2] // 2 == v:
                        put(dst, j, n * KB + 16 * s, _lincomb([(c, src[half, k]) for c, half, k in prod[side]]))

        return [(partial(piece, v, s), pacers) for v in range(5) for s in range(KB // 16)]

    def diag_operands(side, load, dst, pacers, products):
        def piece(e, n, s):
            sub = {(r, m): _lincomb([(c, load(r, half, k, s)) for c, half, k in _PASSES[DIAG + 2 * e + m][n][side]])
                   for r in range(2) for m in range(2)}
            for i in products:
                put(dst, 7 * e + i, n * KB + 16 * s, _strassen_operand(
                    side, i, lambda a, b: sub[a, b] if side == 0 else sub[b, a]))

        return [(partial(piece, e, n, s), pacers) for e in range(2) for n in range(2) for s in range(KB // 16)]

    def transposes(src, dst, pacers, tiles):
        def piece(j):
            put(dst, j, 0, src[j].T)

        return [(partial(piece, j), pacers) for j in tiles] + [(_idle, pacers)]

    def x_operands(u):
        return (pass_operands(0, lambda p, k, s: normalised(2 * u + p, k, s), sx_v, [p_xn])
                + transposes(sx_v, xc_v[u % 2].at[u // 2], [p_sx, p_xc[u % 2]], range(16)))

    def x_diag_operands(b):
        products = (0, 1, 4, 5, 6)
        return (diag_operands(0, lambda r, p, k, s: normalised(4 * b + 2 * r + p, k, s), sp_v, [p_xn], products)
                + transposes(sp_v, xe_v.at[b], [p_sp, p_xe], [7 * e + i for e in range(2) for i in products]))

    def gate_up_operands(i, ft, passes=range(DIAG)):
        slot = i & RING - 1
        return pass_operands(
            1, lambda q, k, s: w_v[slot, 4 * q + ft, block_rows(k, s, 16), :], wc_v.at[ft], [p_w], passes)

    def gate_up_diag_operands(i, fp):
        slot = i & RING - 1
        return diag_operands(
            1, lambda f, q, k, s: w_v[slot, 4 * q + 2 * fp + f, block_rows(k, s, 16), :], we_v.at[fp], [p_w],
            range(7))

    def tile_pair_operands(i, fp):
        return gate_up_diag_operands(i, fp) + gate_up_operands(i, 2 * fp) + gate_up_operands(i, 2 * fp + 1)

    def down_operands(i, slices=range(DR // 16)):
        src = [down_tile(i, k) for k in range(4)]

        def piece(s, outer):
            ops = _strassen2_operands(0, outer, lambda r, k: w_v[(*src[k], tile(r * (DR // 16) + s, 16))])
            for n, val in enumerate(ops):
                wd_v[i, 7 * outer + n, tile(s, 16), :] = val.astype(bf16)

        return [(partial(piece, s, outer), [p_w]) for s in slices for outer in range(7)]

    def hidden_operands(i, b, src=None, slices=range(T // 16)):
        def piece(s, outer):
            ops = _strassen2_operands(1, outer, lambda k, t: h_v[b if src is None else src, k, tile(s, 16), tile(t)])
            for n, val in enumerate(ops):
                hc_v[7 * outer + n, b, i, tile(s, 16), :] = val.astype(bf16)

        return [(partial(piece, s, outer), [p_h]) for s in slices for outer in range(7)]

    def proj_operands(c):
        return (pass_operands(1, lambda q, k, s: w_v[RING + q, c, block_rows(k, s, 16), :], sp_v, [p_w])
                + transposes(sp_v, pc_v.at[:, tile(c, T // 2)], [p_sp, p_pc], range(16)))

    def merge_remainders():
        def piece(q, k):
            w_v[RING + q, 6, block_rows(k), :] = jnp.concatenate(
                [qrem_v[block_rows(k), :].astype(f32)[:, 96 * q:96 * q + 96],
                 orem_v[block_rows(k), :].astype(f32)[:, 32 * q:32 * q + 32]], axis=1).astype(bf16)

        return [(partial(piece, q, k), [p_w]) for q in range(2) for k in range(NK)]

    def gate_up(ft, u, diag=None):
        dst = u // 2 if diag or u > 1 else NB
        for m in range(T // GR):
            c = _recombine(lambda j: dot(xc_v[u % 2][u // 2, j, tile(m, GR // 2), :], wc_v[ft, j]),
                           diag and [part[m][u % 2, ft % 2] for part in diag])
            gate, up = (jnp.concatenate([c[0][q], c[1][q]], axis=1) for q in range(2))
            h_v[dst, ft, tile(m, GR), tile(u % 2, 2 * T)] = jnp.maximum(gate, 0.0) * up

    def x_diag(b, e, i, rows=slice(None)):
        return xc_v[i - 2][b, DIAG + 2 * e + i - 2, rows, :] if i in (2, 3) else xe_v[b, 7 * e + i, rows, :]

    def diagonal(fp, b):
        return [[_strassen_recombine(lambda i: dot(x_diag(b, e, i, tile(m, GR // 2)), we_v[fp, 7 * e + i]))
                 for m in range(T // GR)] for e in range(2)]

    def quad_step(i, carry):
        weaver.add(starts(step_copies(i + 1)), 440)
        weaver.add(tile_pair_operands(i, 1), 90)
        for b in range(NB):
            last = b == NB - 1
            pieces = hidden_operands(i, 0) if last else hidden_operands(i - 1, b + 1)
            if b == 2:
                pieces += hidden_operands(0, 0, NB, [i - 1])
            weaver.add(pieces, 114 if last else 123)
            for fp in range(2):
                diag = diagonal(fp, b)
                if last and fp == 0:
                    weaver.add(tile_pair_operands(i + 1, 0), 102)
                for ft in (2 * fp, 2 * fp + 1):
                    if b == 0 and ft == 3:
                        weaver.add(proj_operands(i) + down_operands(i) + down_operands(0, [i]), 284)
                    gate_up(ft, 2 * b, diag)
                    gate_up(ft, 2 * b + 1, diag)
        weaver.drain()
        wait(step_copies(i + 1))
        return carry

    def first_operands(ft):
        for passes in (range(4), range(4, 16)):
            _run(gate_up_operands(0, ft, passes))

    w0 = [gate_up_copies(0, [ft], RING + ft) for ft in range(4)]
    w1 = gate_up_copies(1, range(4), 0)
    extra = extra_copies(2)
    late = step_copies(1) + wo_copies(1)
    _run(starts(x_copies(0) + w0[0] + x_copies(1)))
    qkv_v[4] = jnp.zeros((3 * D // 2, T), u32)
    wait(x_copies(0))
    _run(x_stats(0) + x_operands(0))

    _run(starts(w0[1] + w0[2]))
    p_w()
    wait(w0[0])
    first_operands(0)
    gate_up(0, 0)

    _run(starts(x_copies(2) + w0[3]))
    p_w()
    wait(x_copies(1) + w0[1])
    first_operands(1)
    gate_up(1, 0)
    _run(x_stats(1) + x_operands(1))
    for ft, u in ((0, 1), (1, 1)):
        gate_up(ft, u)

    _run(starts(x_copies(3, 4, 5)))
    p_x()
    wait(x_copies(2) + w0[2] + w0[3])
    first_operands(2)
    weaver.add(gate_up_operands(0, 3, range(16)), 13)
    weaver.add(x_stats(2) + x_operands(2), 54)
    for ft, u in ((2, 0), (3, 0), (2, 1), (3, 1)):
        gate_up(ft, u)

    _run(starts(x_copies(6, 7)))
    p_x()
    wait(x_copies(3, 4, 5))
    weaver.add(starts(w1 + extra + late), 290)
    for u in range(2, NU):
        pieces = x_stats(u + 1) + x_operands(u + 1) if u < NU - 1 else []
        if u == 2:
            weaver.add(x_diag_operands(0) + x_diag_operands(1), 180)
        if u == 5:
            wait(x_copies(6, 7) + w1)
            weaver.add(x_diag_operands(2), 56)
            weaver.add(gate_up_diag_operands(1, 0), 110)
        if u == 6:
            wait(extra)
            weaver.add(proj_operands(0) + x_diag_operands(3), 118)
        if u == 7:
            weaver.add(merge_remainders() + down_operands(0, [0]), 50)
        weaver.add(pieces, 50)
        for ft in range(4):
            gate_up(ft, u)
            if u == NU - 1 and ft == 0:
                weaver.add(gate_up_operands(1, 0) + gate_up_operands(1, 1), 42)
    weaver.drain()
    wait(late)

    lax.fori_loop(1, NQ, quad_step, None)

    def attention(b, t, g):
        st = {}
        lane = lax.broadcasted_iota(jnp.int32, (8, T), 1)
        stays = [lane < T - DIL * w for w in range(W)]

        def load(slot, part, d):
            return qkv_v[slot, pl.ds((part * D + g * 8 * DH + d) // 2, 8, stride=DH // 2), :]

        def split(word):
            return pltpu.bitcast(word << 16, f32), pltpu.bitcast(word & np.uint32(0xFFFF0000), f32)

        def windows(part, d):
            cur, prev = load(t + 1, part, d), load(t, part, d)
            if t == 0 and part == 2:
                prev = jnp.where(b == 0, jnp.broadcast_to(cur[:, 0:1], cur.shape), prev)
            return [split(cur)] + [split(pltpu.roll(lax.select(stays[w], cur, prev), DIL * w, 1)) for w in range(1, W)]

        def scores(d):
            q0, q1 = split(load(t + 1, 0, d))
            part = [q0 * k0 + q1 * k1 for k0, k1 in windows(1, d)]
            st['logits'] = part if d == 0 else [acc + val for acc, val in zip(st['logits'], part)]

        def softmax():
            logits = [val * DH ** -0.5 for val in st['logits']]
            if t == 0:
                pos = lane + b * (4 * T)
                logits = [jnp.where(pos >= DIL * w, logits[w], -1e9) for w in range(W)]
            top = logits[0]
            for val in logits[1:]:
                top = jnp.maximum(top, val)
            weights = [jnp.exp(val - top) for val in logits]
            inv = 1.0 / sum(weights[1:], weights[0])
            st['probs'] = [val * inv for val in weights]

        def values(d):
            vs = windows(2, d)
            for n in range(2):
                terms = [prob * v[n] for prob, v in zip(st['probs'], vs)]
                o_v[t, pl.ds(g * 8 * DH + d + n, 8, stride=DH), :] = sum(terms[1:], terms[0])

        dims = range(0, DH, 2)
        steps = [partial(scores, d) for d in dims] + [softmax] + [partial(values, d) for d in dims]
        return [(step, [p_qkv, p_o]) for step in steps]

    def context_operands(r):
        return pass_operands(0, lambda p, k, s: o_v[2 * r + p, block_rows(k, s, 16), :], oc_v.at[r], [p_o])

    def block_step(b, carry):
        def halo(n):
            rows = pl.ds(n * KB // 2, KB // 2)
            qkv_v[0, rows, :] = qkv_v[4, rows, :]

        weaver.add(hidden_operands(NQ - 1, b), 250)
        weaver.add([(partial(halo, n), [p_qkv]) for n in range(NK, 3 * NK)], 100)
        for r in range(2):
            if r:
                p_pc()
            for n in range(0, 3 * D // 2, PR):
                c = _recombine(lambda j: dot(pc_v[j, pl.ds(n // 2, PR // 2), :], xc_v[r][b, j], _NT))
                for p in range(2):
                    for q in range(2):
                        row = 6 * T * q + n if n < 6 * T else 12 * T + PR * q
                        put(qkv_v, 1 + 2 * r + p, row, c[p][q])

        pieces = []
        for t in range(4):
            for g in range(H // 8):
                pieces += attention(b, t, g)
            if t % 2:
                pieces += context_operands(t // 2)
        weaver.add(pieces, 49 * NQ - 30)

        def product(j):
            acc = dot(wd_v[0, j], hc_v[j, b, 0], _NT)
            for k in range(1, NQ):
                acc = acc + dot(wd_v[k, j], hc_v[j, b, k], _NT)
            return acc

        started = []
        for outer, (_, _, w) in enumerate(_STRASSEN):
            sub = _strassen_recombine(lambda i: product(7 * outer + i))
            for key in ((0, 0), (0, 1), (1, 0), (1, 1)):
                if w[key]:
                    for (rr, cc), val in sub.items():
                        t, rows = 2 * key[1] + cc, pl.ds((2 * key[0] + rr) * DR, DR)
                        old = y_v[t, rows, :] if key in started else x_v[b, t, rows, :].astype(f32)
                        y_v[t, rows, :] = old + val if w[key] > 0 else old - val
                    started.append(key)
        weaver.drain()

        p_oc()
        p_y()
        for r in range(2):
            p_pc()
            for n in range(0, D // 2, PR):
                c = _recombine(lambda j: dot(pc_v[j, pl.ds((3 * D // 2 + n) // 2, PR // 2), :], oc_v[r, j]))
                for p in range(2):
                    for q in range(2):
                        for row, lo, hi in out_parts(n, q):
                            rows = pl.ds(row, hi - lo)
                            out_v[b, r, rows, tile(p)] = (y_v[2 * r + p, rows, :] + c[p][q][lo:hi]).astype(bf16)
                _run(starts(out_copies(b, r, n)))
        return carry

    lax.fori_loop(0, NB, block_step, None)
    wait([cp for b in range(NB) for r in range(2) for n in range(0, D // 2, PR) for cp in out_copies(b, r, n)])


@jax.jit
def pallas_parallel_sum__sliding_local_dilated__glu_gated_reglu__prompt_kernel(
    A_x: jax.Array,
    A_wqkv: jax.Array,
    A_wo: jax.Array,
    B_x: jax.Array,
    B_W_gate: jax.Array,
    B_W_up: jax.Array,
    B_W_down: jax.Array,
):
    del B_x
    out_t = pl.pallas_call(
        _kernel,
        out_shape=jax.ShapeDtypeStruct((D, S), bf16),
        in_specs=[pl.BlockSpec(memory_space=pl.ANY)] * 6,
        out_specs=pl.BlockSpec(memory_space=pl.ANY),
        scratch_shapes=[
            pltpu.VMEM((NB, 4 + 1, D, T), bf16),
            pltpu.VMEM((RING + 2, 12 + 1, D, T), bf16),
            pltpu.VMEM((D, 3 * D - 12 * T), bf16),
            pltpu.VMEM((D, D - 4 * T), bf16),
            pltpu.VMEM((NB, 2, D, 2 * T), bf16),
            pltpu.VMEM((NB, 16 + 1, T // 2, T), u32),
            pltpu.VMEM((NB, 16 + 1, T // 2, T), u32),
            pltpu.VMEM((NB, 14 + 1, T // 2, T), u32),
            pltpu.VMEM((4, 16, T // 2, T), u32),
            pltpu.VMEM((2, 14, T // 2, T), u32),
            pltpu.VMEM((NQ, 52, DR, T), bf16),
            pltpu.VMEM((49, NB, NQ, T, T), bf16),
            pltpu.VMEM((16 + 1, D, T), u32),
            pltpu.VMEM((2, 16 + 1, T, T), bf16),
            pltpu.VMEM((16 + 1, T, T), bf16),
            pltpu.VMEM((16 + 1, T, T), bf16),
            pltpu.VMEM((S // T + 1, D + 16, T), f32),
            pltpu.VMEM((NB + 1, 4 + 1, T, 4 * T), f32),
            pltpu.VMEM((5 + 1, 3 * D // 2, T), u32),
            pltpu.VMEM((4 + 1, D, T), f32),
            pltpu.VMEM((4 + 1, D, T), f32),
            pltpu.SMEM((1,), jnp.int32),
            pltpu.SemaphoreType.DMA((NU,)),
            pltpu.SemaphoreType.DMA((RING + 4,)),
            pltpu.SemaphoreType.DMA((1,)),
        ],
        compiler_params=pltpu.CompilerParams(
            vmem_limit_bytes=127 * 2**20, disable_bounds_checks=True, disable_semaphore_checks=True),
        name="fused_block",
    )(A_x.reshape(S, D).T, A_wqkv, A_wo, B_W_gate, B_W_up, B_W_down.T)
    return out_t.T.reshape(1, S, D)
```
